```python
import os as _os
_os.environ.setdefault("JAX_PLATFORMS", "cpu")
import jax
import jax.numpy as jnp

def _softmax(x, axis=-1):
    return jax.nn.softmax(x, axis=axis)
def _gelu(x):
    return jax.nn.gelu(x, approximate=True)
def _silu(x):
    return jax.nn.silu(x)
def _sigmoid(x):
    return jax.nn.sigmoid(x)
def _layernorm(x, axis=-1, eps=1e-5):
    m = jnp.mean(x, axis=axis, keepdims=True)
    v = jnp.var(x, axis=axis, keepdims=True)
    return (x - m) / jnp.sqrt(v + eps)
def _scatter_add(tgt, idx, src, axis=0):
    return tgt.at[idx].add(src)
def _segment_sum(src, seg, n):
    return jax.ops.segment_sum(src, seg, n)
class _Rng:
    def __init__(self, key):
        self._k = key
    def _next(self):
        self._k, sub = jax.random.split(self._k)
        return sub
    def normal(self, shape):
        return jax.random.normal(self._next(), shape, dtype=jnp.bfloat16)
    def randint(self, lo, hi, shape):
        return jax.random.randint(self._next(), shape, lo, hi, dtype=jnp.int32)
    def uniform(self, shape, lo=0.0, hi=1.0):
        return jax.random.uniform(self._next(), shape, jnp.bfloat16, lo, hi)
    def permutation(self, n):
        return jax.random.permutation(self._next(), n)


kernel_name = 'standalone__gqa_block_cached__near_ridge'

def setup_inputs():
    _rng = _Rng(jax.random.key(int.from_bytes(__import__("os").urandom(4), "little")))
    _w = (lambda a: (lambda t: t.astype(jnp.bfloat16) if jnp.issubdtype(t.dtype, jnp.floating) else t)(jnp.asarray(a)))
    B, Sq, D = 8, 96, 640
    Hq, Hkv, Sk, Dh = 32, 32, 512, 128
    assert Hq % Hkv == 0, (Hq, Hkv)
    return {
        "x": _w((lambda *s: _rng.normal(s) * 0.2)(B, Sq, D)),
        "k_cache": _w((lambda *s: _rng.normal(s) * 3.2)(B, Hkv, Sk, Dh)),
        "v_cache": _w((lambda *s: _rng.normal(s) * 0.05)(B, Hkv, Sk, Dh)),
        "wq": _w((lambda *s: _rng.normal(s) * 0.2)(D, Hq * Dh) * (D ** -0.5)),
        "wo": _w((lambda *s: _rng.normal(s) * 0.05)(Hq * Dh, D) * ((Hq * Dh) ** -0.5)),
    }

def reference(x, k_cache, v_cache, wq, wo):
    B, Sq, D = x.shape
    Hq, Dh = 32, 128
    Hkv = k_cache.shape[1]
    rep = Hq // Hkv
    q = (lambda x, *d: x.transpose(*d))((x @ wq).reshape(B, Sq, Hq, Dh), 0, 2, 1, 3)
    k = jnp.repeat(k_cache, rep, axis=1)
    v = jnp.repeat(v_cache, rep, axis=1)
    scores = jnp.einsum("bhqd,bhkd->bhqk", q, k) * (Dh ** -0.5)
    p = _softmax(scores, axis=-1)
    o = jnp.einsum("bhqk,bhkd->bhqd", p, v)
    return (lambda x, *d: x.transpose(*d))(o, 0, 2, 1, 3).reshape(B, Sq, Hq * Dh) @ wo
```

```python
import functools

import jax
import jax.numpy as jnp
import jax.experimental.pallas as pl
import jax.experimental.pallas.tpu as pltpu
import numpy as np
from jax import lax

_F32, _BF16 = jnp.float32, jnp.bfloat16
_LOG2E = 1.4426950408889634


@jax.jit
def pallas_standalone__gqa_block_cached__near_ridge_kernel(
    x: jax.Array,
    k_cache: jax.Array,
    v_cache: jax.Array,
    wq: jax.Array,
    wo: jax.Array,
):
    B, Sq, D = x.shape
    _, H, Sk, Dh = k_cache.shape
    assert wq.shape == (D, H * Dh) and wo.shape == (H * Dh, D)
    M = B * Sq
    N = B * H
    G = 4
    NG = H // G
    NC = NG * B
    CR = G * Sk
    PR = 128
    NP = CR // PR
    DA = 3
    R = DA + 1
    WQR = D // B
    WOR = G * Dh // B
    WQ_PR, WO_PR = (32, 32, 16), (24, 24, 16)
    assert sum(WQ_PR) == WQR and sum(WO_PR) == WOR
    NT = D // 128
    L1 = (NG - 1) * B
    ORDER1 = "WAAABBCABCCBCKQQQQOOKOOO"
    ORDER2 = "AAAABBBBCCCCKOOKOOO"
    PAT = "011"
    scale = np.float32((Dh ** -0.5) * _LOG2E)

    def prio(t):
        return int(PAT[t % len(PAT)])

    def kernel_function(x_hbm, k_hbm, v_hbm, wq_hbm, wo_hbm, o_hbm,
                        xb, xnat, wqb, wob, kb, vb, qb, ob, acc, outb,
                        sem, psem, outsem):
        def mo(v, m):
            return v if isinstance(v, int) else pl.multiple_of(v, m)

        def kv_off(i):
            return (i % B) * (H * Sk) + (i // B) * CR

        def kv_rows(i, src, r0, nr, s):
            h, buf = (k_hbm, kb) if src == 0 else (v_hbm, vb)
            return pltpu.make_async_copy(h.at[pl.ds(mo(kv_off(i) + r0, PR), nr)],
                                         buf.at[pl.ds(mo(i * CR + r0, PR), nr)], s)

        def wq_copy(g, r0, nr, s):
            return pltpu.make_async_copy(
                wq_hbm.at[pl.ds(mo(r0, 8), nr), pl.ds(mo(g * G * Dh, G * Dh), G * Dh)],
                wqb.at[g, pl.ds(mo(r0, 8), nr)], s)

        def wo_copy(g, r0, nr, s):
            return pltpu.make_async_copy(wo_hbm.at[pl.ds(mo(g * G * Dh + r0, 8), nr)],
                                         wob.at[g, pl.ds(mo(r0, 8), nr)], s)

        def kv_list(i, s):
            return [functools.partial(kv_rows, i, src, (s0 + j) * PR, PR, s)
                    for s0 in range(0, NP, 2) for src in (0, 1) for j in (0, 1)]

        def has_wq(i):
            return i < (NG - 2) * B

        def has_wo(i):
            return i < (NG - 1) * B

        def wq_list(i, s):
            g, p = i // B + 2, i % B
            out, r = [], 0
            for n in WQ_PR:
                out.append(functools.partial(wq_copy, g, p * WQR + r, n, s))
                r += n
            return out

        def wo_list(i, s):
            g, p = i // B + 1, i % B
            out, r = [], 0
            for n in WO_PR:
                out.append(functools.partial(wo_copy, g, p * WOR + r, n, s))
                r += n
            return out

        def start(lst, pr=None, off=0):
            for t, cp in enumerate(lst):
                cp().start(priority=prio(t + off) if pr is None else pr)

        def when(c):
            if isinstance(c, bool):
                return (lambda f: f()) if c else (lambda f: None)
            return pl.when(c)

        def wait_slot(i, wq_on, wo_on):
            s = sem.at[i % R]
            kv_rows(i, 0, 0, CR, s).wait()
            kv_rows(i, 1, 0, CR, s).wait()

            @when(wq_on)
            def _():
                wq_copy(i // B + 2, (i % B) * WQR, WQR, s).wait()

            @when(wo_on)
            def _():
                wo_copy(i // B + 1, (i % B) * WOR, WOR, s).wait()

        def outcopy(b):
            return pltpu.make_async_copy(outb.at[b], o_hbm.at[pl.ds(mo(b * Sq, Sq), Sq)], outsem)

        def qproj(g, b, heads):
            xx = jnp.concatenate(
                [xb[t, pl.ds(mo(b * Sq, Sq), Sq), :] for t in range(NT)], axis=1)
            for n in heads:
                q = jnp.dot(xx, wqb[g, :, pl.ds(n * Dh, Dh)], preferred_element_type=_F32)
                qb[g * B + b, n] = (q * scale).astype(_BF16)

        XR = 24
        xc = [functools.partial(pltpu.make_async_copy, x_hbm.at[pl.ds(r, XR)],
                                xnat.at[pl.ds(r, XR)], psem.at[0]) for r in range(0, M, XR)]
        wc = [functools.partial(wq_copy, 0, r, 32, psem.at[0]) for r in range(0, D, 32)]
        w1 = [functools.partial(wq_copy, 1, r, 32, psem.at[1]) for r in range(0, D, 32)]
        wo0 = [functools.partial(wo_copy, 0, r, min(24, G * Dh - r), psem.at[1])
               for r in range(0, G * Dh, 24)]
        start(xc + wc, pr=0)
        start(kv_list(0, sem.at[0]), pr=1)
        for cp in xc + wc:
            cp().wait()
        wsl = []
        for i in range(DA):
            wsl += wq_list(i, sem.at[i % R]) + wo_list(i, sem.at[i % R])
        start(w1 + wo0 + wsl)
        for t in range(NT):
            xb[t] = xnat[:, pl.ds(t * 128, 128)]

        def q_first(b, c):
            ch = 1 + b // 4
            start([functools.partial(kv_rows, ch, (t // 2) % 2,
                                     ((2 * (b % 4) + t // 4) * 2 + t % 2) * PR, PR, sem.at[ch % R])
                   for t in range(8)])
            qproj(0, b, range(G))
            return c

        lax.fori_loop(0, B, q_first, 0)
        for cp in w1 + wo0:
            cp().wait()

        def run_ops(order, i, issue_kv, issue_wq, issue_wo, last_group):
            S, P, L = {}, {}, {}
            g, b = i // B, i % B
            cnt = dict(A=0, B=0, C=0, O=0, Q=0, K=0, W=0)
            nxt = i + DA
            ns = sem.at[nxt % R]
            nk = order.count("K")
            nq = order.count("Q")
            for op in order:
                u = cnt[op]
                cnt[op] += 1
                if op == "K":
                    @when(issue_kv)
                    def _():
                        lst = kv_list(nxt, ns)
                        n = len(lst) // nk
                        start(lst[u * n:(u + 1) * n], off=u * n)
                elif op == "W":
                    @when(issue_wq)
                    def _():
                        start(wq_list(nxt, ns))

                    @when(issue_wo)
                    def _():
                        start(wo_list(nxt, ns), off=len(WQ_PR))
                elif op == "A":
                    s = lax.dot_general(qb[i, u], kb[pl.ds(mo(i * CR + u * Sk, Sk), Sk), :],
                                        (((1,), (1,)), ((), ())), preferred_element_type=_F32)
                    S[u] = (s, jnp.max(s, axis=-1, keepdims=True))
                elif op == "B":
                    s, m = S.pop(u)
                    p = jnp.exp2(s - m)
                    l = jnp.sum(p, axis=-1, keepdims=True)
                    r = pl.reciprocal(l, approx=True)
                    L[u] = r * (2.0 - l * r)
                    P[u] = p.astype(_BF16)
                elif op == "C":
                    o = jnp.dot(P.pop(u), vb[pl.ds(mo(i * CR + u * Sk, Sk), Sk), :],
                                preferred_element_type=_F32)
                    ob[u] = (o * L.pop(u)).astype(_BF16)
                elif op == "O":
                    oo = jnp.concatenate([ob[hh] for hh in range(G)], axis=1)
                    cols = pl.ds(u * 128, 128)
                    part = jnp.dot(oo, wob[g, :, cols], preferred_element_type=_F32)
                    if last_group:
                        outb[b, :, cols] = (acc[b, :, cols] + part).astype(_BF16)
                        if u == NT - 1:
                            outcopy(b).start()
                    else:
                        acc[b, :, cols] = jnp.where(g == 0, 0.0, acc[b, :, cols]) + part
                elif op == "Q":
                    hs = G // nq
                    qproj(g + 1, b, range(u * hs, (u + 1) * hs))

        def body1(i, carry):
            wait_slot(i, has_wq(i), True)
            run_ops(ORDER1, i, True, has_wq(i + DA), has_wo(i + DA), False)
            return carry

        def body2(i, carry):
            wait_slot(i, False, False)
            run_ops(ORDER2, i, i + DA < NC, False, False, True)
            return carry

        lax.fori_loop(0, L1, body1, 0)
        lax.fori_loop(L1, NC, body2, 0)
        pltpu.make_async_copy(outb, outb, outsem).wait()

    hbm = pl.BlockSpec(memory_space=pl.ANY)
    out = pl.pallas_call(
        kernel_function,
        out_shape=jax.ShapeDtypeStruct((M, D), x.dtype),
        in_specs=[hbm] * 5,
        out_specs=hbm,
        scratch_shapes=[
            pltpu.VMEM((NT, M, 128), _BF16),
            pltpu.VMEM((M, D), _BF16),
            pltpu.VMEM((NG, D, G * Dh), _BF16),
            pltpu.VMEM((NG, G * Dh, D), _BF16),
            pltpu.VMEM((N * Sk, Dh), _BF16),
            pltpu.VMEM((N * Sk, Dh), _BF16),
            pltpu.VMEM((NC, G, Sq, Dh), _BF16),
            pltpu.VMEM((G, Sq, Dh), _BF16),
            pltpu.VMEM((B, Sq, D), _F32),
            pltpu.VMEM((B, Sq, D), _BF16),
            pltpu.SemaphoreType.DMA((R,)),
            pltpu.SemaphoreType.DMA((2,)),
            pltpu.SemaphoreType.DMA,
        ],
        compiler_params=pltpu.CompilerParams(
            vmem_limit_bytes=110 * 1024 * 1024,
            flags={"XLA_TPU_MAX_INSTS_TO_PREDICATE": 65536},
            disable_bounds_checks=True,
        ),
        name="gqa_block_cached",
    )(x.reshape(M, D), k_cache.reshape(N * Sk, Dh), v_cache.reshape(N * Sk, Dh), wq, wo)
    return out.reshape(B, Sq, D)
```

```python
import functools

import jax
import jax.numpy as jnp
import jax.experimental.pallas as pl
import jax.experimental.pallas.tpu as pltpu
import numpy as np
from jax import lax

_F32, _BF16 = jnp.float32, jnp.bfloat16
_LOG2E = 1.4426950408889634


@jax.jit
def pallas_standalone__gqa_block_cached__near_ridge_kernel(
    x: jax.Array,
    k_cache: jax.Array,
    v_cache: jax.Array,
    wq: jax.Array,
    wo: jax.Array,
):
    B, Sq, D = x.shape
    _, H, Sk, Dh = k_cache.shape
    assert wq.shape == (D, H * Dh) and wo.shape == (H * Dh, D)
    assert v_cache.shape == k_cache.shape and k_cache.shape[0] == B
    M = B * Sq
    N = B * H
    G = 4
    NG = H // G
    NC = NG * B
    CR = G * Sk
    PR = 128
    NP = CR // PR
    DA = 4
    R = DA
    GD = G * Dh
    WQR = D // B
    WOR = GD // B
    WQ_PR, WO_PR = (32, 32, 16), (32, 32)
    assert sum(WQ_PR) == WQR and sum(WO_PR) == WOR
    assert (B, NP, DA) == (8, 16, 4)
    NT = D // 128
    L1 = (NG - 1) * B
    ORDER1 = "AAABBCABCCBCKQQQQWOOKOOO"
    ORDER2 = "AAAABBBBCCCCOOOOOK"
    PAT_KV, PAT_W = "101", "10"
    scale = np.float32((Dh ** -0.5) * _LOG2E)

    def kernel_function(x_hbm, k_hbm, v_hbm, wq_hbm, wo_hbm, o_hbm,
                        xb, xnat, wqb, wob, kb, vb, qb, ob, acc, outb):
        def main(sem, outsem):
            def mo(val, m):
                return val if isinstance(val, int) else pl.multiple_of(val, m)

            def kv_rows(i, src, r0, nr, s):
                h, buf = (k_hbm, kb) if src == 0 else (v_hbm, vb)
                off = (i % B) * (H * Sk) + (i // B) * CR
                return pltpu.make_async_copy(h.at[pl.ds(mo(off + r0, PR), nr)],
                                             buf.at[pl.ds(mo(i * CR + r0, PR), nr)], s)

            def wq_copy(g, r0, nr, s):
                return pltpu.make_async_copy(
                    wq_hbm.at[pl.ds(mo(r0, 8), nr), pl.ds(mo(g * GD, GD), GD)],
                    wqb.at[g, pl.ds(mo(r0, 8), nr)], s)

            def wo_copy(g, r0, nr, s):
                return pltpu.make_async_copy(wo_hbm.at[pl.ds(mo(g * GD + r0, 8), nr)],
                                             wob.at[g, pl.ds(mo(r0, 8), nr)], s)

            def out_copy(b):
                return pltpu.make_async_copy(outb.at[b], o_hbm.at[pl.ds(mo(b * Sq, Sq), Sq)], outsem)

            def piece_index(j, src):
                return (j + src * (NP // 2)) % NP

            def kv_list(i):
                return [functools.partial(kv_rows, i, src, piece_index(j0 + j, src) * PR, PR, sem.at[i % R])
                        for j0 in range(0, NP, 2) for src in (0, 1) for j in (0, 1)]

            def has_wq(i):
                return i < (NG - 2) * B

            def has_wo(i):
                return i < (NG - 1) * B

            def w_list(copy, rows, g, r0, s):
                out = []
                for n in rows:
                    out.append(functools.partial(copy, g, r0, n, s))
                    r0 = r0 + n
                return out

            def wq_list(i):
                return w_list(wq_copy, WQ_PR, i // B + 2, (i % B) * WQR, sem.at[i % R])

            def wo_list(i):
                return w_list(wo_copy, WO_PR, i // B + 1, (i % B) * WOR, sem.at[i % R])

            def start(lst, pat, off=0):
                for t, cp in enumerate(lst):
                    cp().start(priority=int(pat[(t + off) % len(pat)]))

            def when(c):
                if isinstance(c, bool):
                    return (lambda f: f()) if c else (lambda f: None)
                return pl.when(c)

            def wait_slot(i, wq_on, wo_on):
                s = sem.at[i % R]
                kv_rows(i, 0, 0, CR, s).wait()
                kv_rows(i, 1, 0, CR, s).wait()

                @when(wq_on)
                def _():
                    wq_copy(i // B + 2, (i % B) * WQR, WQR, s).wait()

                @when(wo_on)
                def _():
                    wo_copy(i // B + 1, (i % B) * WOR, WOR, s).wait()

            def qproj(g, b, heads):
                xx = jnp.concatenate(
                    [xb[t, pl.ds(mo(b * Sq, Sq), Sq), :] for t in range(NT)], axis=1)
                for n in heads:
                    q = jnp.dot(xx, wqb[g, :, pl.ds(n * Dh, Dh)], preferred_element_type=_F32)
                    qb[g * B + b, n] = (q * scale).astype(_BF16)

            XR = 16
            s_x = outsem
            xc = [functools.partial(pltpu.make_async_copy, x_hbm.at[pl.ds(r, XR)],
                                    xnat.at[pl.ds(r, XR)], s_x) for r in range(0, M, XR)]
            wq0 = [functools.partial(wq_copy, 0, r, 32, s_x) for r in range(0, D, 32)]
            wq1 = [functools.partial(wq_copy, 1, r, 32, outsem) for r in range(0, D, 32)]
            wo0 = [functools.partial(wo_copy, 0, r, 32, outsem) for r in range(0, GD, 32)]
            start(xc + wq0, "0")
            start(kv_list(0), "1")
            for cp in xc + wq0:
                cp().wait()
            wsl = []
            for i in range(DA):
                wsl += wq_list(i) + wo_list(i)
            start(wq1 + wo0 + wsl, PAT_KV)
            for t in range(NT):
                xb[t] = xnat[:, pl.ds(t * 128, 128)]
            start(kv_list(3), PAT_KV)

            def q_first(b, c):
                ch = 1 + b // 4
                start([functools.partial(kv_rows, ch, (t // 2) % 2,
                                         piece_index((2 * (b % 4) + t // 4) * 2 + t % 2, (t // 2) % 2) * PR,
                                         PR, sem.at[ch % R]) for t in range(8)], PAT_KV)
                qproj(0, b, range(G))
                return c

            lax.fori_loop(0, B, q_first, 0)
            for cp in wq1 + wo0:
                cp().wait()

            def run_ops(order, i, last_group):
                S, P, L = {}, {}, {}
                g, b = i // B, i % B
                cnt = dict(A=0, B=0, C=0, O=0, Q=0, K=0, W=0)
                nxt = i + DA
                nk = order.count("K")
                for op in order:
                    u = cnt[op]
                    cnt[op] += 1
                    if op == "K":
                        n = 2 * NP // nk
                        if last_group:
                            @pl.when(nxt < NC - 1)
                            def _():
                                start(kv_list(nxt)[u * n:(u + 1) * n], PAT_KV, off=u * n)

                            @pl.when(nxt == NC - 1)
                            def _():
                                start(kv_list(nxt)[u * n:(u + 1) * n], "1")
                        else:
                            start(kv_list(nxt)[u * n:(u + 1) * n], PAT_KV, off=u * n)
                    elif op == "W":
                        @pl.when(has_wq(nxt))
                        def _():
                            start(wq_list(nxt), PAT_W)

                        @pl.when(has_wo(nxt))
                        def _():
                            start(wo_list(nxt), PAT_W, off=len(WQ_PR))
                    elif op == "A":
                        s = lax.dot_general(qb[i, u], kb[pl.ds(mo(i * CR + u * Sk, Sk), Sk), :],
                                            (((1,), (1,)), ((), ())), preferred_element_type=_F32)
                        S[u] = (s, jnp.max(s, axis=-1, keepdims=True))
                    elif op == "B":
                        s, m = S.pop(u)
                        p = jnp.exp2(s - m)
                        l = jnp.sum(p, axis=-1, keepdims=True)
                        r = pl.reciprocal(l, approx=True)
                        L[u] = r * (2.0 - l * r)
                        P[u] = p.astype(_BF16)
                    elif op == "C":
                        o = jnp.dot(P.pop(u), vb[pl.ds(mo(i * CR + u * Sk, Sk), Sk), :],
                                    preferred_element_type=_F32)
                        ob[u] = (o * L.pop(u)).astype(_BF16)
                    elif op == "O":
                        oo = jnp.concatenate([ob[hh] for hh in range(G)], axis=1)
                        cols = pl.ds(u * 128, 128)
                        part = jnp.dot(oo, wob[g, :, cols], preferred_element_type=_F32)
                        if last_group:
                            outb[b, :, cols] = (acc[b, :, cols] + part).astype(_BF16)
                            if u == NT - 1:
                                @pl.when(i == NC - 1)
                                def _():
                                    out_copy(b).start(priority=1)
                        else:
                            acc[b, :, cols] = jnp.where(g == 0, 0.0, acc[b, :, cols]) + part
                    elif op == "Q":
                        qproj(g + 1, b, [u])

            def body1(i, carry):
                wait_slot(i, has_wq(i), True)
                run_ops(ORDER1, i, False)
                return carry

            def body2(i, carry):
                @pl.when(i == NC - 1)
                def _():
                    for bb in range(B - 1):
                        out_copy(bb).start(priority=1)

                wait_slot(i, False, False)
                run_ops(ORDER2, i, True)
                return carry

            lax.fori_loop(0, L1, body1, 0)
            lax.fori_loop(L1, NC, body2, 0)
            for bb in range(B):
                out_copy(bb).wait()

        pl.run_scoped(main, pltpu.SemaphoreType.DMA((R,)), pltpu.SemaphoreType.DMA)

    hbm = pl.BlockSpec(memory_space=pl.ANY)
    out = pl.pallas_call(
        kernel_function,
        out_shape=jax.ShapeDtypeStruct((M, D), x.dtype),
        in_specs=[hbm] * 5,
        out_specs=hbm,
        scratch_shapes=[
            pltpu.VMEM((NT, M, 128), _BF16),
            pltpu.VMEM((M, D), _BF16),
            pltpu.VMEM((NG, D, GD), _BF16),
            pltpu.VMEM((NG, GD, D), _BF16),
            pltpu.VMEM((N * Sk, Dh), _BF16),
            pltpu.VMEM((N * Sk, Dh), _BF16),
            pltpu.VMEM((NC, G, Sq, Dh), _BF16),
            pltpu.VMEM((G, Sq, Dh), _BF16),
            pltpu.VMEM((B, Sq, D), _F32),
            pltpu.VMEM((B, Sq, D), _BF16),
        ],
        compiler_params=pltpu.CompilerParams(
            vmem_limit_bytes=110 * 1024 * 1024,
            disable_bounds_checks=True,
        ),
        name="gqa_block_cached",
    )(x.reshape(M, D), k_cache.reshape(N * Sk, Dh), v_cache.reshape(N * Sk, Dh), wq, wo)
    return out.reshape(B, Sq, D)
```
